```python
import os as _os
_os.environ.setdefault("JAX_PLATFORMS", "cpu")
import jax
import jax.numpy as jnp

def _softmax(x, axis=-1):
    return jax.nn.softmax(x, axis=axis)
def _gelu(x):
    return jax.nn.gelu(x, approximate=True)
def _silu(x):
    return jax.nn.silu(x)
def _sigmoid(x):
    return jax.nn.sigmoid(x)
def _layernorm(x, axis=-1, eps=1e-5):
    m = jnp.mean(x, axis=axis, keepdims=True)
    v = jnp.var(x, axis=axis, keepdims=True)
    return (x - m) / jnp.sqrt(v + eps)
def _scatter_add(tgt, idx, src, axis=0):
    return tgt.at[idx].add(src)
def _segment_sum(src, seg, n):
    return jax.ops.segment_sum(src, seg, n)
class _Rng:
    def __init__(self, key):
        self._k = key
    def _next(self):
        self._k, sub = jax.random.split(self._k)
        return sub
    def normal(self, shape):
        return jax.random.normal(self._next(), shape, dtype=jnp.bfloat16)
    def randint(self, lo, hi, shape):
        return jax.random.randint(self._next(), shape, lo, hi, dtype=jnp.int32)
    def uniform(self, shape, lo=0.0, hi=1.0):
        return jax.random.uniform(self._next(), shape, jnp.bfloat16, lo, hi)
    def permutation(self, n):
        return jax.random.permutation(self._next(), n)


kernel_name = 'concat_heads__gqa_block_cached__gqa_block_cached__near_ridge'

def setup_inputs():
    _rng = _Rng(jax.random.key(int.from_bytes(__import__("os").urandom(4), "little")))
    _w = (lambda a: (lambda t: t.astype(jnp.bfloat16) if jnp.issubdtype(t.dtype, jnp.floating) else t)(jnp.asarray(a)))
    def _A_setup():
        B, Sq, D = 8, 128, 576
        Hq, Hkv, Sk, Dh = 32, 16, 512, 128
        assert Hq % Hkv == 0, (Hq, Hkv)
        return {
            "x": _w((lambda *s: _rng.normal(s) * 0.8)(B, Sq, D)),
            "k_cache": _w((lambda *s: _rng.normal(s) * 0.8)(B, Hkv, Sk, Dh)),
            "v_cache": _w((lambda *s: _rng.normal(s) * 0.05)(B, Hkv, Sk, Dh)),
            "wq": _w((lambda *s: _rng.normal(s) * 0.8)(D, Hq * Dh) * (D ** -0.5)),
            "wo": _w((lambda *s: _rng.normal(s) * 0.05)(Hq * Dh, D) * ((Hq * Dh) ** -0.5)),
        }
    _A_in = _A_setup()

    def _B_setup():
        B, Sq, D = 8, 128, 576
        Hq, Hkv, Sk, Dh = 32, 16, 512, 128
        assert Hq % Hkv == 0, (Hq, Hkv)
        return {
            "x": _w((lambda *s: _rng.normal(s) * 0.8)(B, Sq, D)),
            "k_cache": _w((lambda *s: _rng.normal(s) * 0.8)(B, Hkv, Sk, Dh)),
            "v_cache": _w((lambda *s: _rng.normal(s) * 0.05)(B, Hkv, Sk, Dh)),
            "wq": _w((lambda *s: _rng.normal(s) * 0.8)(D, Hq * Dh) * (D ** -0.5)),
            "wo": _w((lambda *s: _rng.normal(s) * 0.05)(Hq * Dh, D) * ((Hq * Dh) ** -0.5)),
        }
    _B_in = _B_setup()

    return {
        "A_x": _A_in["x"],
        "A_k_cache": _A_in["k_cache"],
        "A_v_cache": _A_in["v_cache"],
        "A_wq": _A_in["wq"],
        "A_wo": _A_in["wo"],
        "B_x": _B_in["x"],
        "B_k_cache": _B_in["k_cache"],
        "B_v_cache": _B_in["v_cache"],
        "B_wq": _B_in["wq"],
        "B_wo": _B_in["wo"],
    }

def reference(A_x, A_k_cache, A_v_cache, A_wq, A_wo, B_x, B_k_cache, B_v_cache, B_wq, B_wo):
    def _A_ref(x, k_cache, v_cache, wq, wo):
        B, Sq, D = x.shape
        Hq, Dh = 32, 128
        Hkv = k_cache.shape[1]
        rep = Hq // Hkv
        q = (lambda x, *d: x.transpose(*d))((x @ wq).reshape(B, Sq, Hq, Dh), 0, 2, 1, 3)
        k = jnp.repeat(k_cache, rep, axis=1)
        v = jnp.repeat(v_cache, rep, axis=1)
        scores = jnp.einsum("bhqd,bhkd->bhqk", q, k) * (Dh ** -0.5)
        p = _softmax(scores, axis=-1)
        o = jnp.einsum("bhqk,bhkd->bhqd", p, v)
        return (lambda x, *d: x.transpose(*d))(o, 0, 2, 1, 3).reshape(B, Sq, Hq * Dh) @ wo

    def _B_ref(x, k_cache, v_cache, wq, wo):
        B, Sq, D = x.shape
        Hq, Dh = 32, 128
        Hkv = k_cache.shape[1]
        rep = Hq // Hkv
        q = (lambda x, *d: x.transpose(*d))((x @ wq).reshape(B, Sq, Hq, Dh), 0, 2, 1, 3)
        k = jnp.repeat(k_cache, rep, axis=1)
        v = jnp.repeat(v_cache, rep, axis=1)
        scores = jnp.einsum("bhqd,bhkd->bhqk", q, k) * (Dh ** -0.5)
        p = _softmax(scores, axis=-1)
        o = jnp.einsum("bhqk,bhkd->bhqd", p, v)
        return (lambda x, *d: x.transpose(*d))(o, 0, 2, 1, 3).reshape(B, Sq, Hq * Dh) @ wo

    a = _A_ref(A_x, A_k_cache, A_v_cache, A_wq, A_wo)
    b = _B_ref(B_x, B_k_cache, B_v_cache, B_wq, B_wo)
    return jnp.concatenate([a, b], axis=-1)
```

```python
import numpy as np
import jax
import jax.numpy as jnp
import jax.experimental.pallas as pl
import jax.experimental.pallas.tpu as pltpu

B, SQ, D = 8, 128, 576
HQ, HKV, SK, DH = 32, 16, 512, 128
M = B * SQ
C = float(DH ** -0.5 * np.log2(np.e))
KT = 5
bf16 = jnp.bfloat16
f32 = jnp.float32
u32 = jnp.uint32
NT = (((1,), (1,)), ((), ()))
PACK = int('1')
PACKST = int('1')
ORDER = 'KQSOV'
ORDER0 = 'KXQSV'
ORDERL = 'KOSVP'
G0 = int('1')
G1 = int('2')
G2 = int('2')
G3 = int('8')
FLAGS = {k: True for k in 'XLA_TPU_RESCHEDULE_DMA_DONES'.split(",") if k} or None
UNROLL = int('1')
STARTPOS = int('1')


def ld(ref, r0, n):
    if PACK:
        return pltpu.bitcast(ref.bitcast(u32)[r0 // 2:(r0 + n) // 2, :], bf16)
    return ref[r0:r0 + n, :]


def st(ref, r0, val):
    n = val.shape[0]
    if PACKST:
        ref.bitcast(u32)[r0 // 2:(r0 + n) // 2, :] = pltpu.bitcast(val, u32)
    else:
        ref[r0:r0 + n, :] = val


def transpose_x(xT_ref, X_ref, b):
    for kt in range(KT):
        if kt < KT - 1:
            t = ld(xT_ref.at[b], kt * 128, 128)
        else:
            t = jnp.concatenate([ld(xT_ref.at[b], kt * 128, D - 512), jnp.zeros((KT * 128 - D, SQ), bf16)], axis=0)
        st(X_ref.at[kt], b * SQ, t.T)


def qproj(X_ref, w_ref, wi, q_ref, r0, nr):
    lhs = jnp.concatenate([ld(X_ref.at[kt], r0, nr) for kt in range(KT - 1)], axis=1)
    rhs = jnp.concatenate([ld(w_ref.at[wi], 0, 512), ld(w_ref.at[wi + 1], 0, 512)], axis=1)
    q = jnp.dot(lhs, rhs, preferred_element_type=f32)
    rhs4 = jnp.concatenate([ld(w_ref.at[wi], 512, 64), ld(w_ref.at[wi + 1], 512, 64)], axis=1)
    q = q + jnp.dot(ld(X_ref.at[KT - 1], r0, nr)[:, 0:D - 512], rhs4, preferred_element_type=f32)
    q = (q * C).astype(bf16)
    st(q_ref.at[0], r0, q[:, 0:128])
    st(q_ref.at[1], r0, q[:, 128:256])


def qk(q_ref, k_ref, b):
    qb = jnp.concatenate([ld(q_ref.at[0], b * SQ, SQ), ld(q_ref.at[1], b * SQ, SQ)], axis=0)
    return jax.lax.dot_general(qb, ld(k_ref.at[b], 0, SK), NT, preferred_element_type=f32)


def softmax(s):
    m = jnp.max(s, axis=-1, keepdims=True)
    p = jnp.exp2(s - m)
    l = jnp.sum(p, axis=-1, keepdims=True)
    return p.astype(bf16), l


def pv(pl_, v_ref, o_ref, b):
    p, l = pl_
    o = jnp.dot(p, ld(v_ref.at[b], 0, SK), preferred_element_type=f32)
    o = (o * pl.reciprocal(l, approx=True)).astype(bf16)
    st(o_ref.at[0], b * SQ, o[0:SQ])
    st(o_ref.at[1], b * SQ, o[SQ:2 * SQ])


def oproj(o_ref, w_ref, wi, acc_ref, off, b, init=False):
    rhs = jnp.concatenate([ld(o_ref.at[0], b * SQ, SQ), ld(o_ref.at[1], b * SQ, SQ)], axis=1)
    lhs = jnp.concatenate([ld(w_ref.at[wi], 0, D), ld(w_ref.at[wi + 1], 0, D)], axis=1)
    r = jax.lax.dot_general(lhs, rhs, NT, preferred_element_type=f32)
    if init:
        acc_ref[b, off:off + D, :] = r
    else:
        acc_ref[b, off:off + D, :] += r


def _kernel(axT, ak, av, awq, awoT, bxT, bk, bv, bwq, bwoT, out_hbm,
            xa_v, xb_v, XA, XB, kv, w, qA, qB, oA, oB, acc, out_v,
            sem_st, sem_pe, sem_x, osem):
    KVH = (ak, av, bk, bv)
    WH = (awq, awq, awoT, awoT, bwq, bwq, bwoT, bwoT)

    def kv_copy(i, h, slot, b0, nb, sem):
        return pltpu.make_async_copy(KVH[i].at[b0:b0 + nb, h], kv.at[slot, i, b0:b0 + nb], sem)

    def w_copy(i, h, slot, sem):
        r = i % 2
        if isinstance(h, int):
            src = WH[i].at[:, (2 * h + r) * DH:(2 * h + r + 1) * DH]
        else:
            src = WH[i].at[:, pl.ds(pl.multiple_of((2 * h + r) * DH, DH), DH)]
        return pltpu.make_async_copy(src, w.at[slot, i], sem)

    def x_copy(side, b0, nb, sem):
        return pltpu.make_async_copy((axT, bxT)[side].at[b0:b0 + nb], (xa_v, xb_v)[side].at[b0:b0 + nb], sem)

    def start_iter(h, slot):
        hn = jnp.minimum(h + 1, HKV - 1)
        for i, hh in ((2, h), (3, h), (0, hn), (1, hn)):
            kv_copy(i, hh, slot, 0, B, sem_st.at[slot, 0]).start()
        for i, hh in ((0, hn), (1, hn), (2, h), (3, h), (4, hn), (5, hn), (6, h), (7, h)):
            w_copy(i, hh, slot, sem_st.at[slot, 1]).start()

    def wait_iter(slot):
        pltpu.make_async_copy(kv.at[slot], kv.at[slot], sem_st.at[slot, 0]).wait()
        pltpu.make_async_copy(w.at[slot], w.at[slot], sem_st.at[slot, 1]).wait()

    def finalize(b):
        for j in range(2 * D // 128):
            out_v[b, :, j * 128:(j + 1) * 128] = acc[b, j * 128:(j + 1) * 128, :].T.astype(bf16)
        pltpu.make_async_copy(out_v.at[b], out_hbm.at[b], osem.at[b]).start()

    def phase(order, side, slot, first=False, waits=None, xwaits=None, hook=None):
        q_ref, o_ref = (qA, oA) if side == 0 else (qB, oB)
        qn_ref, op_ref = (qB, oB) if side == 0 else (qA, oA)
        X_ref = XB if side == 0 else XA
        wq_i, wo_i, wown_i = (4, 6, 2) if side == 0 else (0, 2, 6)
        off, offown = (D, 0) if side == 0 else (0, D)
        k_ref, v_ref = kv.at[slot, 2 * side], kv.at[slot, 2 * side + 1]
        w_ref = w.at[slot]
        s_ = {}
        for b in range(B):
            if waits and b in waits:
                for c in waits[b]: c.wait()
            for ci, c in enumerate(order):
                if c == "K":
                    s_["s"] = qk(q_ref, k_ref, b)
                elif c == "S":
                    s_["p"] = softmax(s_.pop("s"))
                elif c == "V":
                    pv(s_.pop("p"), v_ref, o_ref, b)
                elif c == "X":
                    transpose_x(xb_v, XB, b)
                elif c == "Q":
                    qproj(X_ref, w_ref, wq_i, qn_ref, b * SQ, SQ)
                elif c == "O":
                    oproj(op_ref, w_ref, wo_i, acc, off, b, init=first)
                elif c == "P":
                    if b > 0:
                        oproj(o_ref, w_ref, wown_i, acc, offown, b - 1)
                        finalize(b - 1)
                    if b == B - 1:
                        oproj(o_ref, w_ref, wown_i, acc, offown, b)
                        finalize(b)
                if hook is not None and b == 0 and ci == 0:
                    hook()

    n = [0]
    def psem():
        n[0] += 1
        return sem_pe.at[n[0] - 1]

    order_start = []
    w0 = {}
    cs = [x_copy(0, 0, G0, psem()), w_copy(0, 0, 1, psem()), w_copy(1, 0, 1, psem())]
    w0[0] = cs; order_start += cs
    for b in range(G0, B, G0):
        c = x_copy(0, b, G0, psem()); w0[b] = [c]; order_start.append(c)
    w1 = {}
    for b in range(0, B, G1):
        cs = [kv_copy(0, 0, 1, b, G1, psem()), kv_copy(1, 0, 1, b, G1, psem()), x_copy(1, b, G1, psem())]
        if b == 0: cs += [w_copy(4, 0, 1, psem()), w_copy(5, 0, 1, psem())]
        w1[b] = cs; order_start += cs
    w2 = {}
    for b in range(0, B, G2):
        cs = [kv_copy(2, 0, 0, b, G2, psem()), kv_copy(3, 0, 0, b, G2, psem())]
        if b == 0: cs += [w_copy(i, hh, 0, psem()) for i, hh in ((0, 1), (1, 1), (2, 0), (3, 0))]
        w2[b] = cs; order_start += cs
    w3 = {}
    for b in range(0, B, G3):
        cs = [kv_copy(0, 1, 0, b, G3, psem()), kv_copy(1, 1, 0, b, G3, psem())]
        if b == 0: cs += [w_copy(i, hh, 0, psem()) for i, hh in ((4, 1), (5, 1), (6, 0), (7, 0))]
        w3[b] = cs; order_start += cs
    for c in order_start: c.start()

    for b in range(B):
        if b in w0:
            for c in w0[b]: c.wait()
        transpose_x(xa_v, XA, b)
        qproj(XA, w.at[1], 0, qA, b * SQ, SQ)
    phase(ORDER0, 0, 1, waits=w1)
    start_iter(1, 1)
    phase(ORDER, 1, 0, first=True, waits=w2)
    phase(ORDER, 0, 0, first=True, waits=w3)

    def iteration(h):
        slot = h % 2
        wait_iter(slot)
        if STARTPOS == 0:
            start_iter(h + 1, 1 - slot)
            phase(ORDER, 1, slot)
        else:
            phase(ORDER, 1, slot, hook=lambda: start_iter(h + 1, 1 - slot))
        phase(ORDER, 0, slot)

    def body(i, _):
        for u in range(UNROLL):
            iteration(1 + i * UNROLL + u)
        return None

    nit = (HKV - 2) // UNROLL
    assert nit * UNROLL == HKV - 2
    jax.lax.fori_loop(0, nit, body, None)
    wait_iter(1)
    phase(ORDERL, 1, 1)
    for b in range(B):
        pltpu.make_async_copy(out_v.at[b], out_hbm.at[b], osem.at[b]).wait()


@jax.jit
def pallas_concat_heads__gqa_block_cached__gqa_block_cached__near_ridge_kernel(A_x, A_k_cache, A_v_cache, A_wq, A_wo, B_x, B_k_cache, B_v_cache, B_wq, B_wo):
    AxT = jnp.swapaxes(A_x, 1, 2)
    BxT = jnp.swapaxes(B_x, 1, 2)
    any_spec = pl.BlockSpec(memory_space=pltpu.HBM)
    return pl.pallas_call(
        _kernel,
        in_specs=[any_spec] * 10,
        out_specs=any_spec,
        out_shape=jax.ShapeDtypeStruct((B, SQ, 2 * D), bf16),
        scratch_shapes=[pltpu.VMEM((B, D, SQ), bf16), pltpu.VMEM((B, D, SQ), bf16),
                        pltpu.VMEM((KT, M, 128), bf16), pltpu.VMEM((KT, M, 128), bf16),
                        pltpu.VMEM((2, 4, B, SK, DH), bf16), pltpu.VMEM((2, 8, D, DH), bf16),
                        pltpu.VMEM((2, M, DH), bf16), pltpu.VMEM((2, M, DH), bf16),
                        pltpu.VMEM((2, M, DH), bf16), pltpu.VMEM((2, M, DH), bf16),
                        pltpu.VMEM((B, 2 * D, SQ), f32), pltpu.VMEM((B, SQ, 2 * D), bf16),
                        pltpu.SemaphoreType.DMA((2, 2)), pltpu.SemaphoreType.DMA((80,)),
                        pltpu.SemaphoreType.DMA((2,)), pltpu.SemaphoreType.DMA((B,))],
        compiler_params=pltpu.CompilerParams(vmem_limit_bytes=100 * 1024 * 1024, disable_bounds_checks=bool(int('1')), disable_semaphore_checks=bool(int('1')), flags=FLAGS),
    )(AxT, A_k_cache, A_v_cache, A_wq, A_wo.T, BxT, B_k_cache, B_v_cache, B_wq, B_wo.T)
```

```python
import contextlib
import numpy as np
import jax
import jax.numpy as jnp
import jax.experimental.pallas as pl
import jax.experimental.pallas.tpu as pltpu

B, SQ, D = 8, 128, 576
HQ, HKV, SK, DH = 32, 16, 512, 128
M = B * SQ
C = float(DH ** -0.5 * np.log2(np.e))
KT = 5
bf16 = jnp.bfloat16
f32 = jnp.float32
u32 = jnp.uint32
NT = (((1,), (1,)), ((), ()))
PACK = int('1')
PACKST = int('1')
ORDER = 'twrKeQSEOWRV'
ORDER0 = 'wrKxeXQSWRV'
ORDERL = 'wK|EOSWVPf'
FLAGS = {k: True for k in 'XLA_TPU_RESCHEDULE_DMA_DONES'.split(",") if k} or None
LAG = int('1')
SEPW = int('1')
BAR0 = int('1')
BARS = [int(c) for c in '46']
SEPO = int('1')
BF16T = int('1')
NODMA = int('0')
G = int('2')
SCOPES = int('0')


def scope(name):
    return jax.named_scope(name) if SCOPES else contextlib.nullcontext()


def ld(ref, r0, n):
    if PACK:
        return pltpu.bitcast(ref.bitcast(u32)[r0 // 2:(r0 + n) // 2, :], bf16)
    return ref[r0:r0 + n, :]


def st(ref, r0, val):
    n = val.shape[0]
    if PACKST:
        ref.bitcast(u32)[r0 // 2:(r0 + n) // 2, :] = pltpu.bitcast(val, u32)
    else:
        ref[r0:r0 + n, :] = val


def transpose_x(xT_ref, X_ref, b):
    for kt in range(KT):
        if kt < KT - 1:
            t = ld(xT_ref.at[b], kt * 128, 128)
        else:
            t = jnp.concatenate([ld(xT_ref.at[b], kt * 128, D - 512), jnp.zeros((KT * 128 - D, SQ), bf16)], axis=0)
        st(X_ref.at[kt], b * SQ, t.T)


def qproj(X_ref, w_ref, q_ref, r0, nr):
    lhs = jnp.concatenate([ld(X_ref.at[kt], r0, nr) for kt in range(KT - 1)], axis=1)
    rhs = jnp.concatenate([ld(w_ref.at[0], 0, 512), ld(w_ref.at[1], 0, 512)], axis=1)
    q = jnp.dot(lhs, rhs, preferred_element_type=f32)
    rhs4 = jnp.concatenate([ld(w_ref.at[0], 512, 64), ld(w_ref.at[1], 512, 64)], axis=1)
    q = q + jnp.dot(ld(X_ref.at[KT - 1], r0, nr)[:, 0:D - 512], rhs4, preferred_element_type=f32)
    q = (q * C).astype(bf16)
    st(q_ref.at[0], r0, q[:, 0:128])
    st(q_ref.at[1], r0, q[:, 128:256])


def qk(q_ref, k_ref, b):
    qb = jnp.concatenate([ld(q_ref.at[0], b * SQ, SQ), ld(q_ref.at[1], b * SQ, SQ)], axis=0)
    return jax.lax.dot_general(qb, ld(k_ref.at[b], 0, SK), NT, preferred_element_type=f32)


def softmax(s):
    m = jnp.max(s, axis=-1, keepdims=True)
    p = jnp.exp2(s - m)
    l = jnp.sum(p, axis=-1, keepdims=True)
    return p.astype(bf16), l


def pv(pl_, v_ref, o_ref, b):
    p, l = pl_
    o = jnp.dot(p, ld(v_ref.at[b], 0, SK), preferred_element_type=f32)
    o = (o * pl.reciprocal(l, approx=True)).astype(bf16)
    st(o_ref.at[0], b * SQ, o[0:SQ])
    st(o_ref.at[1], b * SQ, o[SQ:2 * SQ])


def oproj(o_ref, w_ref, acc_ref, off, b):
    rhs = jnp.concatenate([ld(o_ref.at[0], b * SQ, SQ), ld(o_ref.at[1], b * SQ, SQ)], axis=1)
    lhs = jnp.concatenate([ld(w_ref.at[0], 0, D), ld(w_ref.at[1], 0, D)], axis=1)
    r = jax.lax.dot_general(lhs, rhs, NT, preferred_element_type=f32)
    acc_ref[b, off:off + D, :] += r


def _kernel(axT, ak, av, awq, awoT, bxT, bk, bv, bwq, bwoT, out_hbm,
            xa_v, xb_v, XA, XB, kA, vA, kB, vB, wqA, woA, wqB, woB, qA, qB, oA, oB, acc, out_v, woL,
            sems, sem_w, bsem, osem, wq0):
    KH = (ak, bk); VH = (av, bv); KV = (kA, kB); VV = (vA, vB)
    WQH = (awq, bwq); WOH = (awoT, bwoT); WQ = (wqA, wqB); WO = (woA, woB)
    XX = (XA, XB); QQ = (qA, qB); OO = (oA, oB)

    def k_copy(side, h, b, g=1):
        return pltpu.make_async_copy(KH[side].at[b:b + g, h], KV[side].at[b:b + g], sems.at[side * 16 + b])

    def v_copy(side, h, b, g=1):
        return pltpu.make_async_copy(VH[side].at[b:b + g, h], VV[side].at[b:b + g], sems.at[side * 16 + 8 + b])

    def w_copies(src, dst, h, si, init=False):
        out = []
        for r in range(2):
            if isinstance(h, int):
                s = src.at[:, (2 * h + r) * DH:(2 * h + r + 1) * DH]
            else:
                s = src.at[:, pl.ds(pl.multiple_of((2 * h + r) * DH, DH), DH)]
            out.append(pltpu.make_async_copy(s, dst.at[r], (sems.at[32 + si * 2 + r] if (init or not SEPW) else sem_w.at[si * 2 + r])))
        return out

    def wq_copies(side, h, init=False): return w_copies(WQH[side], WQ[side], h, side, init)
    def wo_copies(side, h): return w_copies(WOH[side], WO[side], h, 2 + side)

    def wl_copies(): return w_copies(bwoT, woL, HKV - 1, 4, True)

    def x_copy(side, b):
        return pltpu.make_async_copy((axT, bxT)[side].at[b], (xa_v, xb_v)[side].at[b], sems.at[42 + side * 8 + b])

    def out_copy(b):
        return pltpu.make_async_copy(out_v.at[b], out_hbm.at[b], (osem.at[b] if SEPO else sems.at[58 + b]))

    class _Nop:
        def start(self): pass
        def wait(self): pass
    if NODMA:
        k_copy = v_copy = x_copy = lambda *a: _Nop()
        w_copies = lambda *a: [_Nop()]

    def start(cs):
        for c in cs: c.start()

    def wait(cs):
        for c in cs: c.wait()

    def barrier():
        pl.semaphore_signal(bsem, 1)
        pl.semaphore_wait(bsem, 1)

    def finalize(b):
        for j in range(2 * D // 128):
            if BF16T:
                out_v[b, :, j * 128:(j + 1) * 128] = acc[b, j * 128:(j + 1) * 128, :].astype(bf16).T
            else:
                out_v[b, :, j * 128:(j + 1) * 128] = acc[b, j * 128:(j + 1) * 128, :].T.astype(bf16)

    def phase(order, side, h, hq, ho, nh=None, nhq=None, nho=None):
        other = 1 - side
        gw = 1 if order == ORDER0 else G
        off, offown = (D, 0) if side == 0 else (0, D)
        s_ = {}
        for b in range(B):
          with (scope(f"s1_step{b}") if order == ORDER0 and SCOPES > 1 else contextlib.nullcontext()):
            for c in order:
                if c == "w":
                    if b % gw == 0: k_copy(side, h, b, gw).wait()
                elif c == "W":
                    if b % gw == 0: v_copy(side, h, b, gw).wait()
                elif c == "r":
                    if nh is not None and b % G == 0: k_copy(other, nh, b, G).start()
                elif c == "R":
                    if nh is not None and b % G == 0: v_copy(other, nh, b, G).start()
                elif c == "t":
                    if b == 0:
                        if nhq is not None: start(wq_copies(side, nhq))
                        if nho is not None: start(wo_copies(side, nho))
                elif c == "e":
                    if b == 0: wait(wq_copies(other, hq, order == ORDER0))
                elif c == "E":
                    if b == 0:
                        wait(wo_copies(other, ho))
                elif c == "K":
                    s_["s"] = qk(QQ[side], KV[side], b)
                elif c == "S":
                    s_["p"] = softmax(s_.pop("s"))
                elif c == "V":
                    pv(s_.pop("p"), VV[side], OO[side], b)
                elif c == "z":
                    acc[b] = jnp.zeros(acc.shape[1:], f32)
                elif c == "x":
                    x_copy(other, b).wait()
                elif c == "X":
                    transpose_x((xa_v, xb_v)[other], XX[other], b)
                elif c == "Q":
                    qproj(XX[other], WQ[other], QQ[other], b * SQ, SQ)
                elif c == "O":
                    oproj(OO[other], WO[other], acc, off, b)
                elif c == "|":
                    if b in BARS: barrier()
                elif c == "f":
                    if b >= LAG: out_copy(b - LAG).start()
                elif c == "P":
                    if b == 1: wait(wl_copies())
                    if b > 0:
                        oproj(OO[side], woL, acc, offown, b - 1)
                        finalize(b - 1)
                    if b == B - 1:
                        for bb in range(B - LAG, B - 1): out_copy(bb).start()
                        oproj(OO[side], woL, acc, offown, b)
                        finalize(b)
                        out_copy(b).start()

    start(w_copies(awq, wq0, 0, 0, True))
    for b in range(0, B): x_copy(0, b).start()
    for b in range(B):
        k_copy(0, 0, b).start(); x_copy(1, b).start()
        if b == 0: start(wq_copies(1, 0, True))
        v_copy(0, 0, b).start()
    start(wo_copies(0, 0))
    start(wq_copies(0, 1))

    acc[...] = jnp.zeros(acc.shape, f32)
    if BAR0: barrier()
    with scope("s0_QA0"):
        for b in range(B):
            x_copy(0, b).wait()
            if b == 0: wait(w_copies(awq, wq0, 0, 0, True))
            transpose_x(xa_v, XA, b)
            qproj(XA, wq0, qA, b * SQ, SQ)
    with scope("s1_P1p"):
        phase(ORDER0, 0, 0, 0, None, nh=0)

    def body(h, _):
        with scope("s4_iter"):
            phase(ORDER, 1, h, h + 1, h, nh=h + 1, nhq=h + 1, nho=h)
            phase(ORDER, 0, h + 1, h + 1, h, nh=h + 1, nhq=jnp.minimum(h + 2, HKV - 1), nho=h + 1)
        return None

    jax.lax.fori_loop(0, HKV - 1, body, None)
    with scope("s5_epi"):
        start(wl_copies())
        phase(ORDERL, 1, HKV - 1, None, HKV - 1)
        wait(wq_copies(0, HKV - 1))
    with scope("s6_outwait"):
        for b in range(B):
            out_copy(b).wait()


@jax.jit
def pallas_concat_heads__gqa_block_cached__gqa_block_cached__near_ridge_kernel(A_x, A_k_cache, A_v_cache, A_wq, A_wo, B_x, B_k_cache, B_v_cache, B_wq, B_wo):
    AxT = jnp.swapaxes(A_x, 1, 2)
    BxT = jnp.swapaxes(B_x, 1, 2)
    any_spec = pl.BlockSpec(memory_space=pltpu.HBM)
    wshape = pltpu.VMEM((2, D, DH), bf16)
    kvshape = pltpu.VMEM((B, SK, DH), bf16)
    return pl.pallas_call(
        _kernel,
        in_specs=[any_spec] * 10,
        out_specs=any_spec,
        out_shape=jax.ShapeDtypeStruct((B, SQ, 2 * D), bf16),
        scratch_shapes=[pltpu.VMEM((B, D, SQ), bf16), pltpu.VMEM((B, D, SQ), bf16),
                        pltpu.VMEM((KT, M, 128), bf16), pltpu.VMEM((KT, M, 128), bf16),
                        kvshape, kvshape, kvshape, kvshape, wshape, wshape, wshape, wshape,
                        pltpu.VMEM((2, M, DH), bf16), pltpu.VMEM((2, M, DH), bf16),
                        pltpu.VMEM((2, M, DH), bf16), pltpu.VMEM((2, M, DH), bf16),
                        pltpu.VMEM((B, 2 * D, SQ), f32), pltpu.VMEM((B, SQ, 2 * D), bf16), wshape,
                        pltpu.SemaphoreType.DMA((66,)), pltpu.SemaphoreType.DMA((10,)), pltpu.SemaphoreType.REGULAR, pltpu.SemaphoreType.DMA((B,)), wshape],
        compiler_params=pltpu.CompilerParams(vmem_limit_bytes=100 * 1024 * 1024, disable_bounds_checks=True,
                                             disable_semaphore_checks=bool(int('1')), flags=FLAGS),
    )(AxT, A_k_cache, A_v_cache, A_wq, A_wo.T, BxT, B_k_cache, B_v_cache, B_wq, B_wo.T)
```

```python
import contextlib
import numpy as np
import jax
import jax.numpy as jnp
import jax.experimental.pallas as pl
import jax.experimental.pallas.tpu as pltpu

B, SQ, D = 8, 128, 576
HQ, HKV, SK, DH = 32, 16, 512, 128
M = B * SQ
C = float(DH ** -0.5 * np.log2(np.e))
KT = 5
bf16 = jnp.bfloat16
f32 = jnp.float32
u32 = jnp.uint32
NT = (((1,), (1,)), ((), ()))
PACK = int('1')
PACKST = int('1')
ORDER = 'twrKQSOWRVn'
ORDER0 = 'xeXwrRKQSWVn'
ORDERL = 'wK|OSWVPf'
OFIRST = 'tQwrKSOWRV'
OLAST = '' or ORDER
OMID0 = '' or ORDER
OMID7 = '' or ORDER
FLAGS = {k: True for k in 'XLA_TPU_RESCHEDULE_DMA_DONES'.split(",") if k} or None
LAG = int('1')
SEPW = int('1')
BAR0 = int('1')
BARS = [int(c) for c in '6']
SEPO = int('1')
BF16T = int('1')
NODMA = int('0')
G = int('2')
INITO = 'xkwv'
XFIRST = int('0')
NBAR = int('1')
SCOPES = int('0')


def scope(name):
    return jax.named_scope(name) if SCOPES else contextlib.nullcontext()


def ld(ref, r0, n):
    if PACK:
        return pltpu.bitcast(ref.bitcast(u32)[r0 // 2:(r0 + n) // 2, :], bf16)
    return ref[r0:r0 + n, :]


def st(ref, r0, val):
    n = val.shape[0]
    if PACKST:
        ref.bitcast(u32)[r0 // 2:(r0 + n) // 2, :] = pltpu.bitcast(val, u32)
    else:
        ref[r0:r0 + n, :] = val


def transpose_x(xT_ref, X_ref, b):
    for kt in range(KT):
        if kt < KT - 1:
            t = ld(xT_ref.at[b], kt * 128, 128)
        else:
            t = jnp.concatenate([ld(xT_ref.at[b], kt * 128, D - 512), jnp.zeros((KT * 128 - D, SQ), bf16)], axis=0)
        st(X_ref.at[kt], b * SQ, t.T)


def qproj(X_ref, w_ref, q_ref, r0, nr):
    lhs = jnp.concatenate([ld(X_ref.at[kt], r0, nr) for kt in range(KT - 1)], axis=1)
    rhs = jnp.concatenate([ld(w_ref.at[0], 0, 512), ld(w_ref.at[1], 0, 512)], axis=1)
    q = jnp.dot(lhs, rhs, preferred_element_type=f32)
    rhs4 = jnp.concatenate([ld(w_ref.at[0], 512, 64), ld(w_ref.at[1], 512, 64)], axis=1)
    q = q + jnp.dot(ld(X_ref.at[KT - 1], r0, nr)[:, 0:D - 512], rhs4, preferred_element_type=f32)
    q = (q * C).astype(bf16)
    st(q_ref.at[0], r0, q[:, 0:128])
    st(q_ref.at[1], r0, q[:, 128:256])


def qk(q_ref, k_ref, b):
    qb = jnp.concatenate([ld(q_ref.at[0], b * SQ, SQ), ld(q_ref.at[1], b * SQ, SQ)], axis=0)
    return jax.lax.dot_general(qb, ld(k_ref.at[b], 0, SK), NT, preferred_element_type=f32)


def softmax(s):
    m = jnp.max(s, axis=-1, keepdims=True)
    p = jnp.exp2(s - m)
    l = jnp.sum(p, axis=-1, keepdims=True)
    return p.astype(bf16), l


def pv(pl_, v_ref, o_ref, b):
    p, l = pl_
    o = jnp.dot(p, ld(v_ref.at[b], 0, SK), preferred_element_type=f32)
    o = (o * pl.reciprocal(l, approx=True)).astype(bf16)
    st(o_ref.at[0], b * SQ, o[0:SQ])
    st(o_ref.at[1], b * SQ, o[SQ:2 * SQ])


def oproj(o_ref, w_ref, acc_ref, off, b):
    rhs = jnp.concatenate([ld(o_ref.at[0], b * SQ, SQ), ld(o_ref.at[1], b * SQ, SQ)], axis=1)
    lhs = jnp.concatenate([ld(w_ref.at[0], 0, D), ld(w_ref.at[1], 0, D)], axis=1)
    r = jax.lax.dot_general(lhs, rhs, NT, preferred_element_type=f32)
    acc_ref[b, off:off + D, :] += r


def _kernel(axT, ak, av, awq, awoT, bxT, bk, bv, bwq, bwoT, out_hbm,
            xa_v, xb_v, XA, XB, kA, vA, kB, vB, wqA, woA, wqB, woB, qA, qB, oA, oB, acc, out_v, woL,
            sems, sem_w, bsem, osem, wq0):
    KH = (ak, bk); VH = (av, bv); KV = (kA, kB); VV = (vA, vB)
    WQH = (awq, bwq); WOH = (awoT, bwoT); WQ = (wqA, wqB); WO = (woA, woB)
    XX = (XA, XB); QQ = (qA, qB); OO = (oA, oB)

    def k_copy(side, h, b, g=1):
        return pltpu.make_async_copy(KH[side].at[b:b + g, h], KV[side].at[b:b + g], sems.at[side * 16 + b])

    def v_copy(side, h, b, g=1):
        return pltpu.make_async_copy(VH[side].at[b:b + g, h], VV[side].at[b:b + g], sems.at[side * 16 + 8 + b])

    def w_copies(src, dst, h, si, init=False):
        out = []
        for r in range(2):
            if isinstance(h, int):
                s = src.at[:, (2 * h + r) * DH:(2 * h + r + 1) * DH]
            else:
                s = src.at[:, pl.ds(pl.multiple_of((2 * h + r) * DH, DH), DH)]
            out.append(pltpu.make_async_copy(s, dst.at[r], (sems.at[32 + si * 2 + r] if (init or not SEPW) else sem_w.at[si * 2 + r])))
        return out

    def wq_copies(side, h, init=False): return w_copies(WQH[side], WQ[side], h, side, init)
    def wo_copies(side, h): return w_copies(WOH[side], WO[side], h, 2 + side)

    def wl_copies(): return w_copies(bwoT, woL, HKV - 1, 4, True)

    def x_copy(side, b):
        return pltpu.make_async_copy((axT, bxT)[side].at[b], (xa_v, xb_v)[side].at[b], sems.at[42 + side * 8 + b])

    def out_copy(b):
        return pltpu.make_async_copy(out_v.at[b], out_hbm.at[b], (osem.at[b] if SEPO else sems.at[58 + b]))

    class _Nop:
        def start(self): pass
        def wait(self): pass
    if NODMA:
        k_copy = v_copy = x_copy = lambda *a: _Nop()
        w_copies = lambda *a: [_Nop()]

    def start(cs):
        for c in cs: c.start()

    def wait(cs):
        for c in cs: c.wait()

    def barrier():
        pl.semaphore_signal(bsem, 1)
        pl.semaphore_wait(bsem, 1)

    def finalize(b):
        for j in range(2 * D // 128):
            if BF16T:
                out_v[b, :, j * 128:(j + 1) * 128] = acc[b, j * 128:(j + 1) * 128, :].astype(bf16).T
            else:
                out_v[b, :, j * 128:(j + 1) * 128] = acc[b, j * 128:(j + 1) * 128, :].T.astype(bf16)

    def phase(order, side, h, hq, ho, nh=None, nhq=None, nho=None, wq_next=None, wo_next=None):
        other = 1 - side
        gw = 1 if order == ORDER0 else G
        off, offown = (D, 0) if side == 0 else (0, D)
        s_ = {}
        if wq_next is None: wq_next, wo_next = nhq, nho
        for b in range(B):
          with (scope(f"s1_step{b}") if order == ORDER0 and SCOPES > 1 else contextlib.nullcontext()):
            ordb = order
            if order == ORDER:
                if side == 1 and b == 0: ordb = OFIRST
                if side == 0 and b == B - 1: ordb = OLAST
                if side == 0 and b == 0: ordb = OMID0
                if side == 1 and b == B - 1: ordb = OMID7
            for c in ordb:
                if c == "w":
                    if b % gw == 0: k_copy(side, h, b, gw).wait()
                elif c == "W":
                    if b % gw == 0: v_copy(side, h, b, gw).wait()
                elif c == "r":
                    if nh is not None and b % G == 0: k_copy(other, nh, b, G).start()
                elif c == "R":
                    if nh is not None and b % G == 0: v_copy(other, nh, b, G).start()
                elif c == "t":
                    if b == 0:
                        if nhq is not None: start(wq_copies(side, nhq))
                        if nho is not None: start(wo_copies(side, nho))
                elif c == "n":
                    if b == B - 1:
                        if side == 0 and NBAR: barrier()
                        wait(wq_copies(side, wq_next)); wait(wo_copies(side, wo_next))
                elif c == "e":
                    if b == 0: wait(wq_copies(other, hq, order == ORDER0))
                elif c == "E":
                    if b == 0:
                        wait(wo_copies(other, ho))
                elif c == "K":
                    s_["s"] = qk(QQ[side], KV[side], b)
                elif c == "S":
                    s_["p"] = softmax(s_.pop("s"))
                elif c == "V":
                    pv(s_.pop("p"), VV[side], OO[side], b)
                elif c == "z":
                    acc[b] = jnp.zeros(acc.shape[1:], f32)
                elif c == "x":
                    x_copy(other, b).wait()
                elif c == "X":
                    transpose_x((xa_v, xb_v)[other], XX[other], b)
                elif c == "Q":
                    qproj(XX[other], WQ[other], QQ[other], b * SQ, SQ)
                elif c == "O":
                    oproj(OO[other], WO[other], acc, off, b)
                elif c == "|":
                    if b in BARS: barrier()
                elif c == "f":
                    if b >= LAG: out_copy(b - LAG).start()
                elif c == "P":
                    if b == 1: wait(wl_copies())
                    if b > 0:
                        oproj(OO[side], woL, acc, offown, b - 1)
                        finalize(b - 1)
                    if b == B - 1:
                        for bb in range(B - LAG, B - 1): out_copy(bb).start()
                        oproj(OO[side], woL, acc, offown, b)
                        finalize(b)
                        out_copy(b).start()

    for b in range(0, B):
        if b == XFIRST: start(w_copies(awq, wq0, 0, 0, True))
        x_copy(0, b).start()
    for b in range(B):
        for c in INITO:
            if c == "k": k_copy(0, 0, b).start()
            if c == "x": x_copy(1, b).start()
            if c == "w" and b == 0: start(wq_copies(1, 0, True))
            if c == "v": v_copy(0, 0, b).start()
    start(wo_copies(0, 0))
    start(wq_copies(0, 1))

    acc[...] = jnp.zeros(acc.shape, f32)
    if BAR0: barrier()
    with scope("s0_QA0"):
        for b in range(B):
            x_copy(0, b).wait()
            if b == 0: wait(w_copies(awq, wq0, 0, 0, True))
            transpose_x(xa_v, XA, b)
            qproj(XA, wq0, qA, b * SQ, SQ)
    with scope("s1_P1p"):
        phase(ORDER0, 0, 0, 0, None, nh=0, wq_next=1, wo_next=0)

    def body(h, _):
        with scope("s4_iter"):
            phase(ORDER, 1, h, h + 1, h, nh=h + 1, nhq=h + 1, nho=h)
            phase(ORDER, 0, h + 1, h + 1, h, nh=h + 1, nhq=jnp.minimum(h + 2, HKV - 1), nho=h + 1)
        return None

    jax.lax.fori_loop(0, HKV - 1, body, None)
    with scope("s5_epi"):
        start(wl_copies())
        phase(ORDERL, 1, HKV - 1, None, HKV - 1)
    with scope("s6_outwait"):
        for b in range(B):
            out_copy(b).wait()


@jax.jit
def pallas_concat_heads__gqa_block_cached__gqa_block_cached__near_ridge_kernel(A_x, A_k_cache, A_v_cache, A_wq, A_wo, B_x, B_k_cache, B_v_cache, B_wq, B_wo):
    AxT = jnp.swapaxes(A_x, 1, 2)
    BxT = jnp.swapaxes(B_x, 1, 2)
    any_spec = pl.BlockSpec(memory_space=pltpu.HBM)
    wshape = pltpu.VMEM((2, D, DH), bf16)
    kvshape = pltpu.VMEM((B, SK, DH), bf16)
    return pl.pallas_call(
        _kernel,
        in_specs=[any_spec] * 10,
        out_specs=any_spec,
        out_shape=jax.ShapeDtypeStruct((B, SQ, 2 * D), bf16),
        scratch_shapes=[pltpu.VMEM((B, D, SQ), bf16), pltpu.VMEM((B, D, SQ), bf16),
                        pltpu.VMEM((KT, M, 128), bf16), pltpu.VMEM((KT, M, 128), bf16),
                        kvshape, kvshape, kvshape, kvshape, wshape, wshape, wshape, wshape,
                        pltpu.VMEM((2, M, DH), bf16), pltpu.VMEM((2, M, DH), bf16),
                        pltpu.VMEM((2, M, DH), bf16), pltpu.VMEM((2, M, DH), bf16),
                        pltpu.VMEM((B, 2 * D, SQ), f32), pltpu.VMEM((B, SQ, 2 * D), bf16), wshape,
                        pltpu.SemaphoreType.DMA((66,)), pltpu.SemaphoreType.DMA((10,)), pltpu.SemaphoreType.REGULAR, pltpu.SemaphoreType.DMA((B,)), wshape],
        compiler_params=pltpu.CompilerParams(vmem_limit_bytes=100 * 1024 * 1024, disable_bounds_checks=True,
                                             disable_semaphore_checks=bool(int('1')), flags=FLAGS),
    )(AxT, A_k_cache, A_v_cache, A_wq, A_wo.T, BxT, B_k_cache, B_v_cache, B_wq, B_wo.T)
```

```python
import numpy as np
import jax
import jax.numpy as jnp
import jax.experimental.pallas as pl
import jax.experimental.pallas.tpu as pltpu

B, SQ, D = 8, 128, 576
HQ, HKV, SK, DH = 32, 16, 512, 128
M = B * SQ
C = float(DH ** -0.5 * np.log2(np.e))
KT = 5
G = 2
bf16 = jnp.bfloat16
f32 = jnp.float32
u32 = jnp.uint32
NT = (((1,), (1,)), ((), ()))

ORDER = "twrKQSOWRVn"
ORDER_FIRST = "tQwrKSOWRV"
ORDER_PRO = "xeXwrRKQSWVn"
ORDER_EPI = "wK|OSWVPf"
EPI_BARRIER = 6


def _ld(ref, r0, n):
    return pltpu.bitcast(ref.bitcast(u32)[r0 // 2:(r0 + n) // 2, :], bf16)


def _st(ref, r0, val):
    ref[r0:r0 + val.shape[0], :] = val


def _transpose_x(xT_ref, X_ref, b):
    for kt in range(KT):
        if kt < KT - 1:
            t = _ld(xT_ref.at[b], kt * 128, 128)
        else:
            t = jnp.concatenate([_ld(xT_ref.at[b], kt * 128, D - 512),
                                 jnp.zeros((KT * 128 - D, SQ), bf16)], axis=0)
        _st(X_ref.at[kt], b * SQ, t.T)


def _qproj(X_ref, w_ref, q_ref, b):
    r0 = b * SQ
    lhs = jnp.concatenate([_ld(X_ref.at[kt], r0, SQ) for kt in range(KT - 1)], axis=1)
    rhs = jnp.concatenate([_ld(w_ref.at[0], 0, 512), _ld(w_ref.at[1], 0, 512)], axis=1)
    q = jnp.dot(lhs, rhs, preferred_element_type=f32)
    rhs4 = jnp.concatenate([_ld(w_ref.at[0], 512, 64), _ld(w_ref.at[1], 512, 64)], axis=1)
    q = q + jnp.dot(_ld(X_ref.at[KT - 1], r0, SQ)[:, 0:D - 512], rhs4, preferred_element_type=f32)
    q = (q * C).astype(bf16)
    _st(q_ref.at[0], r0, q[:, 0:DH])
    _st(q_ref.at[1], r0, q[:, DH:2 * DH])


def _qk(q_ref, k_ref, b):
    qb = jnp.concatenate([_ld(q_ref.at[0], b * SQ, SQ), _ld(q_ref.at[1], b * SQ, SQ)], axis=0)
    return jax.lax.dot_general(qb, _ld(k_ref.at[b], 0, SK), NT, preferred_element_type=f32)


def _softmax(s):
    m = jnp.max(s, axis=-1, keepdims=True)
    p = jnp.exp2(s - m)
    l = jnp.sum(p, axis=-1, keepdims=True)
    return p.astype(bf16), l


def _pv(p_l, v_ref, o_ref, b):
    p, l = p_l
    o = jnp.dot(p, _ld(v_ref.at[b], 0, SK), preferred_element_type=f32)
    o = (o * pl.reciprocal(l, approx=True)).astype(bf16)
    _st(o_ref.at[0], b * SQ, o[0:SQ])
    _st(o_ref.at[1], b * SQ, o[SQ:2 * SQ])


def _oproj(o_ref, w_ref, acc_ref, off, b):
    rhs = jnp.concatenate([_ld(o_ref.at[0], b * SQ, SQ), _ld(o_ref.at[1], b * SQ, SQ)], axis=1)
    lhs = jnp.concatenate([_ld(w_ref.at[0], 0, D), _ld(w_ref.at[1], 0, D)], axis=1)
    acc_ref[b, off:off + D, :] += jax.lax.dot_general(lhs, rhs, NT, preferred_element_type=f32)


def _kernel(axT, ak, av, awq, awoT, bxT, bk, bv, bwq, bwoT, out_hbm,
            xa_v, xb_v, XA, XB, kA, vA, kB, vB, wqA, woA, wqB, woB, qA, qB, oA, oB, acc, out_v, woL,
            sems, sem_w, bsem, osem, wq0):
    KH = (ak, bk); VH = (av, bv); KV = (kA, kB); VV = (vA, vB)
    WQH = (awq, bwq); WOH = (awoT, bwoT); WQ = (wqA, wqB); WO = (woA, woB)
    XX = (XA, XB); QQ = (qA, qB); OO = (oA, oB)

    def k_copy(side, h, b, g=1):
        return pltpu.make_async_copy(KH[side].at[b:b + g, h], KV[side].at[b:b + g], sems.at[side * 16 + b])

    def v_copy(side, h, b, g=1):
        return pltpu.make_async_copy(VH[side].at[b:b + g, h], VV[side].at[b:b + g], sems.at[side * 16 + 8 + b])

    def w_copies(src, dst, h, si, once=False):
        out = []
        for r in range(2):
            if isinstance(h, int):
                s = src.at[:, (2 * h + r) * DH:(2 * h + r + 1) * DH]
            else:
                s = src.at[:, pl.ds(pl.multiple_of((2 * h + r) * DH, DH), DH)]
            sem = sems.at[32 + si * 2 + r] if once else sem_w.at[si * 2 + r]
            out.append(pltpu.make_async_copy(s, dst.at[r], sem))
        return out

    def wq_copies(side, h, once=False): return w_copies(WQH[side], WQ[side], h, side, once)
    def wo_copies(side, h): return w_copies(WOH[side], WO[side], h, 2 + side)
    def wl_copies(): return w_copies(bwoT, woL, HKV - 1, 4, True)

    def x_copy(side, b):
        return pltpu.make_async_copy((axT, bxT)[side].at[b], (xa_v, xb_v)[side].at[b], sems.at[42 + side * 8 + b])

    def out_copy(b):
        return pltpu.make_async_copy(out_v.at[b], out_hbm.at[b], osem.at[b])

    def start(cs):
        for c in cs: c.start()

    def wait(cs):
        for c in cs: c.wait()

    def barrier():
        pl.semaphore_signal(bsem, 1)
        pl.semaphore_wait(bsem, 1)

    def finalize(b):
        for j in range(2 * D // 128):
            out_v[b, :, j * 128:(j + 1) * 128] = acc[b, j * 128:(j + 1) * 128, :].astype(bf16).T

    def phase(order, side, h, nh=None, nhq=None, nho=None, prefetch_w=True):
        other = 1 - side
        gw = 1 if order == ORDER_PRO else G
        off, offown = (D, 0) if side == 0 else (0, D)
        live = {}
        for b in range(B):
            ordb = ORDER_FIRST if (order == ORDER and side == 1 and b == 0) else order
            for c in ordb:
                if c == "w":
                    if b % gw == 0: k_copy(side, h, b, gw).wait()
                elif c == "W":
                    if b % gw == 0: v_copy(side, h, b, gw).wait()
                elif c == "r":
                    if b % G == 0: k_copy(other, nh, b, G).start()
                elif c == "R":
                    if b % G == 0: v_copy(other, nh, b, G).start()
                elif c == "t":
                    if b == 0:
                        start(wq_copies(side, nhq)); start(wo_copies(side, nho))
                elif c == "n":
                    if b == B - 1:
                        if side == 0: barrier()
                        wait(wq_copies(side, nhq)); wait(wo_copies(side, nho))
                elif c == "e":
                    if b == 0: wait(wq_copies(other, 0, True))
                elif c == "K":
                    live["s"] = _qk(QQ[side], KV[side], b)
                elif c == "S":
                    live["p"] = _softmax(live.pop("s"))
                elif c == "V":
                    _pv(live.pop("p"), VV[side], OO[side], b)
                elif c == "x":
                    x_copy(other, b).wait()
                elif c == "X":
                    _transpose_x((xa_v, xb_v)[other], XX[other], b)
                elif c == "Q":
                    _qproj(XX[other], WQ[other], QQ[other], b)
                elif c == "O":
                    _oproj(OO[other], WO[other], acc, off, b)
                elif c == "|":
                    if b == EPI_BARRIER: barrier()
                elif c == "f":
                    if 1 <= b < B - 1: out_copy(b - 1).start()
                elif c == "P":
                    if b == 1: wait(wl_copies())
                    if b > 0:
                        _oproj(OO[side], woL, acc, offown, b - 1)
                        finalize(b - 1)
                    if b == B - 1:
                        _oproj(OO[side], woL, acc, offown, b)
                        finalize(b)
                        out_copy(b).start()
                        out_copy(b - 1).start()

    start(w_copies(awq, wq0, 0, 0, True))
    for b in range(B): x_copy(0, b).start()
    for b in range(B):
        x_copy(1, b).start()
        k_copy(0, 0, b).start()
        if b == 0: start(wq_copies(1, 0, True))
        v_copy(0, 0, b).start()
    start(wo_copies(0, 0))
    start(wq_copies(0, 1))
    acc[...] = jnp.zeros(acc.shape, f32)
    barrier()

    for b in range(B):
        x_copy(0, b).wait()
        if b == 0: wait(w_copies(awq, wq0, 0, 0, True))
        _transpose_x(xa_v, XA, b)
        _qproj(XA, wq0, qA, b)
    phase(ORDER_PRO, 0, 0, nh=0, nhq=1, nho=0)

    def body(h, _):
        phase(ORDER, 1, h, nh=h + 1, nhq=h + 1, nho=h)
        phase(ORDER, 0, h + 1, nh=h + 1, nhq=jnp.minimum(h + 2, HKV - 1), nho=h + 1)
        return None

    jax.lax.fori_loop(0, HKV - 1, body, None)

    start(wl_copies())
    phase(ORDER_EPI, 1, HKV - 1)
    for b in range(B):
        out_copy(b).wait()


@jax.jit
def pallas_concat_heads__gqa_block_cached__gqa_block_cached__near_ridge_kernel(
    A_x: jax.Array,
    A_k_cache: jax.Array,
    A_v_cache: jax.Array,
    A_wq: jax.Array,
    A_wo: jax.Array,
    B_x: jax.Array,
    B_k_cache: jax.Array,
    B_v_cache: jax.Array,
    B_wq: jax.Array,
    B_wo: jax.Array,
):
    hbm = pl.BlockSpec(memory_space=pltpu.HBM)
    wshape = pltpu.VMEM((2, D, DH), bf16)
    kvshape = pltpu.VMEM((B, SK, DH), bf16)
    hshape = pltpu.VMEM((2, M, DH), bf16)
    return pl.pallas_call(
        _kernel,
        in_specs=[hbm] * 10,
        out_specs=hbm,
        out_shape=jax.ShapeDtypeStruct((B, SQ, 2 * D), bf16),
        scratch_shapes=[pltpu.VMEM((B, D, SQ), bf16), pltpu.VMEM((B, D, SQ), bf16),
                        pltpu.VMEM((KT, M, 128), bf16), pltpu.VMEM((KT, M, 128), bf16),
                        kvshape, kvshape, kvshape, kvshape, wshape, wshape, wshape, wshape,
                        hshape, hshape, hshape, hshape,
                        pltpu.VMEM((B, 2 * D, SQ), f32), pltpu.VMEM((B, SQ, 2 * D), bf16), wshape,
                        pltpu.SemaphoreType.DMA((58,)), pltpu.SemaphoreType.DMA((8,)),
                        pltpu.SemaphoreType.REGULAR, pltpu.SemaphoreType.DMA((B,)), wshape],
        compiler_params=pltpu.CompilerParams(
            vmem_limit_bytes=64 * 1024 * 1024,
            disable_bounds_checks=True,
            disable_semaphore_checks=True,
            flags={"XLA_TPU_RESCHEDULE_DMA_DONES": True},
        ),
    )(jnp.swapaxes(A_x, 1, 2), A_k_cache, A_v_cache, A_wq, A_wo.T,
      jnp.swapaxes(B_x, 1, 2), B_k_cache, B_v_cache, B_wq, B_wo.T)
```
